```python
import os as _os
_os.environ.setdefault('JAX_PLATFORMS', 'cpu')
import jax
import jax.numpy as jnp

def _softmax(x, axis=-1):
    return jax.nn.softmax(x, axis=axis)

def _gelu(x):
    return jax.nn.gelu(x, approximate=True)

def _silu(x):
    return jax.nn.silu(x)

def _sigmoid(x):
    return jax.nn.sigmoid(x)

def _layernorm(x, axis=-1, eps=1e-05):
    m = jnp.mean(x, axis=axis, keepdims=True)
    v = jnp.var(x, axis=axis, keepdims=True)
    return (x - m) / jnp.sqrt(v + eps)

def _scatter_add(tgt, idx, src, axis=0):
    return tgt.at[idx].add(src)

def _segment_sum(src, seg, n):
    return jax.ops.segment_sum(src, seg, n)

class _Rng:

    def __init__(self, key):
        self._k = key

    def _next(self):
        self._k, sub = jax.random.split(self._k)
        return sub

    def normal(self, shape):
        return jax.random.normal(self._next(), shape, dtype=jnp.bfloat16)

    def randint(self, lo, hi, shape):
        return jax.random.randint(self._next(), shape, lo, hi, dtype=jnp.int32)

    def uniform(self, shape, lo=0.0, hi=1.0):
        return jax.random.uniform(self._next(), shape, jnp.bfloat16, lo, hi)

    def permutation(self, n):
        return jax.random.permutation(self._next(), n)
kernel_name = 'gated_mix__memory_aug_recurrent_mem_tr__glu_gated_geglu__prompt'

def setup_inputs():
    _rng = _Rng(jax.random.key(int.from_bytes(__import__("os").urandom(4), "little")))
    _w = lambda a: (lambda t: t.astype(jnp.bfloat16) if jnp.issubdtype(t.dtype, jnp.floating) else t)(jnp.asarray(a))

    def _A_setup():
        B, S, Dm = (1, 2048, 640)
        H, Dh = (32, 128)
        M, seg = (8, 32)
        seg = min(seg, S)
        S = S // seg * seg
        return {'x': _w((lambda *s: _rng.normal(s) * 0.05)(B, S, Dm)), 'mem0': _w((lambda *s: _rng.normal(s) * 0.4)(B, M, Dm)), 'Wq': _w((lambda *s: _rng.normal(s) * 3.2)(Dm, H, Dh) * Dm ** (-0.5)), 'Wk': _w((lambda *s: _rng.normal(s) * 3.2)(Dm, H, Dh) * Dm ** (-0.5)), 'Wv': _w((lambda *s: _rng.normal(s) * 0.4)(Dm, H, Dh) * Dm ** (-0.5)), 'Wo': _w((lambda *s: _rng.normal(s) * 0.4)(H, Dh, Dm) * (H * Dh) ** (-0.5)), 'seg_len': seg}
    _A_in = _A_setup()

    def _B_setup():
        B, S, Dm, Df = (1, 2048, 640, 1728)
        return {'x': _w((lambda *s: _rng.normal(s) * 0.05)(B, S, Dm)), 'w_gate': _w((lambda *s: _rng.normal(s) * 1.6)(Dm, Df) * Dm ** (-0.5)), 'w_up': _w((lambda *s: _rng.normal(s) * 1.6)(Dm, Df) * Dm ** (-0.5)), 'w_down': _w((lambda *s: _rng.normal(s) * 1.6)(Df, Dm) * Df ** (-0.5))}
    _B_in = _B_setup()
    return {'A_x': _A_in['x'], 'A_mem0': _A_in['mem0'], 'A_Wq': _A_in['Wq'], 'A_Wk': _A_in['Wk'], 'A_Wv': _A_in['Wv'], 'A_Wo': _A_in['Wo'], 'A_seg_len': _A_in['seg_len'], 'B_x': _B_in['x'], 'B_w_gate': _B_in['w_gate'], 'B_w_up': _B_in['w_up'], 'B_w_down': _B_in['w_down'], 'gate_w': _w((lambda *s: _rng.normal(s) * 0.05)(640) * 16.0)}

def reference(A_x, A_mem0, A_Wq, A_Wk, A_Wv, A_Wo, A_seg_len, B_x, B_w_gate, B_w_up, B_w_down, gate_w):

    def _A_ref(x, mem0, Wq, Wk, Wv, Wo, seg_len):
        B, S, Dm = x.shape
        H, Dh = (Wq.shape[1], Wq.shape[2])
        M = mem0.shape[1]
        scale = Dh ** (-0.5)
        n_seg = S // seg_len
        L = M + seg_len
        idx = jnp.arange(L)
        mask = (idx[:, None] < M) | (idx[:, None] >= idx[None, :])
        mem = mem0
        outs = []
        for s in range(n_seg):
            xs = x[:, s * seg_len:(s + 1) * seg_len, :].copy()
            h = jnp.concatenate([mem, xs], axis=1)
            q = jnp.einsum('btd,dhe->bhte', h, Wq)
            k = jnp.einsum('btd,dhe->bhte', h, Wk)
            v = jnp.einsum('btd,dhe->bhte', h, Wv)
            scores = jnp.einsum('bhqe,bhke->bhqk', q, k) * scale
            scores = jnp.where(mask[None, None], scores, -1000000000.0)
            p = _softmax(scores, axis=-1)
            o = jnp.einsum('bhqk,bhke->bhqe', p, v)
            o = jnp.einsum('bhte,hed->btd', o, Wo)
            mem = o[:, :M, :].copy()
            outs.append(o[:, M:, :])
        return jnp.concatenate(outs, axis=1)

    def _B_ref(x, w_gate, w_up, w_down):
        g = jnp.einsum('bsd,df->bsf', x, w_gate)
        u = jnp.einsum('bsd,df->bsf', x, w_up)
        h = _gelu(g) * u
        return jnp.einsum('bsf,fd->bsd', h, w_down)
    x = A_x
    g = _sigmoid((x * gate_w).sum(-1, keepdims=True))
    a = _A_ref(x, A_mem0, A_Wq, A_Wk, A_Wv, A_Wo, A_seg_len)
    b = _B_ref(x, B_w_gate, B_w_up, B_w_down)
    return g * a + (1 - g) * b
```

```python
import jax
import jax.numpy as jnp
import numpy as np
import jax.experimental.pallas as pl
import jax.experimental.pallas.tpu as pltpu

S, DM, H, DH, M, SEG, DF = 2048, 640, 32, 128, 8, 32, 1728
NSEG = S // SEG
LP = 48
FB = S // (H // 2)
F32, BF16 = jnp.float32, jnp.bfloat16


def _dot(a, b):
    return jnp.dot(a, b, preferred_element_type=F32)


def _kernel(x_hbm, mem_ref, wq_hbm, wk_hbm, wv_hbm, wo_hbm, wg_hbm, wu_hbm, wd_hbm, gw_ref,
            o_ref,
            x_v, wraw, wqkv, wo_v, wg_v, wu_v, wd_v, b_v, g_v, h_v, sems):
    cps = [pltpu.make_async_copy(s, d, sems.at[i]) for i, (s, d) in enumerate((
        (x_hbm, x_v), (wg_hbm, wg_v), (wu_hbm, wu_v), (wd_hbm, wd_v),
        (wq_hbm, wraw.at[0]), (wk_hbm, wraw.at[1]), (wv_hbm, wraw.at[2]), (wo_hbm, wo_v)))]
    for c in cps:
        c.start()
    for c in cps[:4]:
        c.wait()

    def ffn(i, c):
        r = pl.ds(pl.multiple_of(i * FB, FB), FB)
        xb = x_v[r, :]
        g = _dot(xb, wg_v[...])
        u = _dot(xb, wu_v[...])
        hh = (jax.nn.gelu(g, approximate=True) * u).astype(BF16)
        b = _dot(hh, wd_v[...])
        gate = jax.nn.sigmoid(jnp.sum(xb.astype(F32) * gw_ref[...].astype(F32), axis=-1, keepdims=True))
        b_v[r, :] = (1.0 - gate) * b
        g_v[r, :] = jnp.broadcast_to(gate, (FB, DH))
        return c

    jax.lax.fori_loop(0, H // 2, ffn, 0)
    for c in cps[4:7]:
        c.wait()

    def relayout(j, c):
        for t in range(3):
            w = wraw.at[t].bitcast(jnp.uint32)[:, j, :]
            lo = pltpu.bitcast(w << 16, F32).astype(BF16)
            hi = pltpu.bitcast(w & jnp.uint32(0xFFFF0000), F32).astype(BF16)
            wqkv[2 * j, :, t * DH:(t + 1) * DH] = lo
            wqkv[2 * j + 1, :, t * DH:(t + 1) * DH] = hi
        return c

    jax.lax.fori_loop(0, H // 2, relayout, 0)
    cps[7].wait()

    h_v[SEG:, :] = jnp.concatenate([mem_ref[...].astype(F32), jnp.zeros((LP - SEG - M, DM), F32)], 0).astype(BF16)
    qi = jax.lax.broadcasted_iota(jnp.int32, (LP, LP), 0)
    kj = jax.lax.broadcasted_iota(jnp.int32, (LP, LP), 1)
    allowed = (kj < SEG + M) & ((qi >= SEG) | (kj >= SEG) | (kj <= qi))
    fill = jnp.where(kj < SEG + M, -1e9, -jnp.inf).astype(F32)
    scale = DH ** -0.5

    def step(s, c):
        r = pl.ds(pl.multiple_of(s * SEG, SEG), SEG)
        h_v[:SEG, :] = x_v[r, :]
        hb = h_v[...]
        acc = jnp.zeros((LP, DM), F32)
        for hd in range(H):
            qkv = _dot(hb, wqkv[hd])
            q = qkv[:, :DH].astype(BF16)
            k = qkv[:, DH:2 * DH].astype(BF16)
            v = qkv[:, 2 * DH:].astype(BF16)
            sc = jax.lax.dot_general(q, k, (((1,), (1,)), ((), ())), preferred_element_type=F32) * scale
            sc = jnp.where(allowed, sc, fill)
            p = jnp.exp(sc - jnp.max(sc, axis=-1, keepdims=True))
            p = p / jnp.sum(p, axis=-1, keepdims=True)
            o = _dot(p.astype(BF16), v).astype(BF16)
            acc = acc + _dot(o, wo_v[hd * DH:(hd + 1) * DH, :])
        gate = g_v[r, :]
        gate = jnp.concatenate([gate] * (DM // DH), axis=1)
        o_ref[r, :] = (gate * acc[:SEG] + b_v[r, :]).astype(o_ref.dtype)
        h_v[SEG:, :] = jnp.concatenate([acc[SEG:SEG + M], jnp.zeros((LP - SEG - M, DM), F32)], 0).astype(BF16)
        return c

    jax.lax.fori_loop(0, NSEG, step, 0)


@jax.jit
def pallas_gated_mix__memory_aug_recurrent_mem_tr__glu_gated_geglu__prompt_kernel(
    A_x, A_mem0, A_Wq, A_Wk, A_Wv, A_Wo, A_seg_len, B_x, B_w_gate, B_w_up, B_w_down, gate_w,
):
    anyspec = pl.BlockSpec(memory_space=pl.ANY)
    vspec = pl.BlockSpec(memory_space=pltpu.VMEM)
    out = pl.pallas_call(
        _kernel,
        out_shape=jax.ShapeDtypeStruct((S, DM), A_x.dtype),
        in_specs=[anyspec, vspec] + [anyspec] * 7 + [vspec],
        out_specs=vspec,
        scratch_shapes=[
            pltpu.VMEM((S, DM), BF16),
            pltpu.VMEM((3, DM, H, DH), BF16),
            pltpu.VMEM((H, DM, 3 * DH), BF16),
            pltpu.VMEM((H * DH, DM), BF16),
            pltpu.VMEM((DM, DF), BF16),
            pltpu.VMEM((DM, DF), BF16),
            pltpu.VMEM((DF, DM), BF16),
            pltpu.VMEM((S, DM), F32),
            pltpu.VMEM((S, DH), F32),
            pltpu.VMEM((LP, DM), BF16),
            pltpu.SemaphoreType.DMA((8,)),
        ],
        compiler_params=pltpu.CompilerParams(vmem_limit_bytes=110 * 2**20),
    )(A_x.reshape(S, DM), A_mem0.reshape(M, DM), A_Wq, A_Wk, A_Wv, A_Wo.reshape(H * DH, DM),
      B_w_gate, B_w_up, B_w_down, gate_w.reshape(1, DM))
    return out.reshape(1, S, DM)
```

```python
import jax
import jax.numpy as jnp
import numpy as np
import jax.experimental.pallas as pl
import jax.experimental.pallas.tpu as pltpu

S, DM, H, DH, M, SEG, DF = 2048, 640, 32, 128, 8, 32, 1728
NSEG = S // SEG
LP = 48
FB = S // (H // 2)
D1, D2, DP, D3 = 1, 2, 2, 3
T = M
A = SEG - T
N1, G = 8, 4
EC = 4
F32, BF16, U32 = jnp.float32, jnp.bfloat16, jnp.uint32


def _dot(a, b):
    return jnp.dot(a, b, preferred_element_type=F32)


def _dot_nt(a, b):
    return jax.lax.dot_general(a, b, (((1,), (1,)), ((), ())), preferred_element_type=F32)


def _bf(w):
    return pltpu.bitcast(w, BF16)


def _kernel(x_hbm, mem_ref, wq_hbm, wk_hbm, wv_hbm, wo_hbm, wg_hbm, wu_hbm, wd_hbm, gw_ref,
            o_hbm,
            x_v, wraw, wqkv, wo_v, wg_v, wu_v, wd_v, b_v, g_v, xt_v, pre, ot_v, m_v, o_v, sems):
    u32 = lambda r: r.bitcast(U32)
    cps = [pltpu.make_async_copy(s, d, sems.at[i]) for i, (s, d) in enumerate((
        (x_hbm.at[:FB], x_v.at[:FB]), (u32(wg_hbm), wg_v), (u32(wu_hbm), wu_v), (u32(wd_hbm), wd_v),
        (x_hbm.at[FB:], x_v.at[FB:]), (u32(wo_hbm), wo_v)))]
    wcps = [pltpu.make_async_copy(u32(w).at[:, p, j, :], wraw.at[j, p, :, pl.ds(t * DH, DH)], sems.at[6])
            for t, w in enumerate((wq_hbm, wk_hbm, wv_hbm)) for j in range(H // 2) for p in range(2)]
    for c in cps[:5]:
        c.start()

    def ffn(i, hook=lambda k: None):
        r = pl.ds(pl.multiple_of(i * FB, FB), FB)
        hook(0)
        xb = x_v[r, :]
        xf = xb.astype(F32)
        for k in range(FB // SEG):
            xt_v[pl.ds(pl.multiple_of(i * (FB // SEG * T) + k * T, T), T), :] = xf[k * SEG + A:(k + 1) * SEG]
        gate = jax.nn.sigmoid(jnp.sum(xf * gw_ref[...].astype(F32), axis=-1, keepdims=True))
        hook(1)
        g = _dot_nt(xb, _bf(wg_v[...]))
        hook(2)
        u = _dot_nt(xb, _bf(wu_v[...]))
        hh = (jax.nn.gelu(g, approximate=True) * u).astype(BF16)
        hook(3)
        b_v[r, :] = (1.0 - gate) * _dot(hh, _bf(wd_v[...]))
        g_v[r, :] = jnp.broadcast_to(gate, (FB, DH))

    def repack(base, j):
        gi, c0 = base + 2 * j // G, 2 * j % G * 3 * DH
        e, o = wraw[base * (G // 2) + j, 0], wraw[base * (G // 2) + j, 1]
        wqkv[gi, :, c0:c0 + 3 * DH] = (e & jnp.uint32(0xFFFF)) | (o << 16)
        wqkv[gi, :, c0 + 3 * DH:c0 + 6 * DH] = (e >> 16) | (o & jnp.uint32(0xFFFF0000))

    def first(k):
        cps[k].wait()
        if k == 3:
            for c in wcps + [cps[5]]:
                c.start()

    ffn(0, first)
    cps[4].wait()
    jax.lax.fori_loop(1, N1, lambda i, c: ffn(i), None)
    pltpu.make_async_copy(wraw, wraw, sems.at[6]).wait()

    def ffn_repack(i, c):
        ffn(i + N1)
        for k in range((G // 2)):
            repack(i, k)

    jax.lax.fori_loop(0, H // 2 // (G // 2), ffn_repack, None)
    if N1 + H // 2 // (G // 2) < S // FB:
        jax.lax.fori_loop(N1 + H // 2 // (G // 2), S // FB, lambda i, c: ffn(i), None)

    def pre_qkv(hd, c):
        xt = xt_v[...].astype(BF16)
        r = _dot(xt, _bf(wqkv[hd])).reshape(NSEG, T, 3 * DH * G)
        pre[hd] = jnp.concatenate([r, jnp.zeros_like(r)], axis=1).astype(BF16)
        return c

    jax.lax.fori_loop(0, H // G, pre_qkv, None)
    cps[5].wait()
    m_v[...] = mem_ref[...].astype(F32)

    qi = jax.lax.broadcasted_iota(jnp.int32, (LP, LP), 0)
    kj = jax.lax.broadcasted_iota(jnp.int32, (LP, LP), 1)
    is_mem = lambda i: (i >= A) & (i < SEG)
    allowed = (kj < SEG + T) & (is_mem(qi) | is_mem(kj) | (kj <= qi))
    fill = jnp.where(kj < SEG + T, -1e9, -jnp.inf).astype(F32)
    scale = DH ** -0.5

    def step(s, c):
        r = pl.multiple_of(s * SEG, SEG)
        hb = jnp.concatenate([x_v[pl.ds(r, SEG), :].astype(F32)[:A], m_v[...]], axis=0).astype(BF16)
        acc = jnp.zeros((SEG, DM), F32)
        st = {}
        NG = H // G
        for t in range(NG + D3):
            if t < NG:
                qkv = jnp.concatenate([_dot(hb, _bf(wqkv[t])).astype(BF16), pre[t, s]], axis=0)
                st[t] = [[qkv[:, (3 * i + j) * DH:(3 * i + j + 1) * DH] for j in range(3)] for i in range(G)]
            if 0 <= t - D1 < NG:
                st[t - D1] = [(_dot_nt(q, k) * scale, v) for q, k, v in st[t - D1]]
            if 0 <= t - D2 < NG:
                os_ = []
                for sc, v in st[t - D2]:
                    sc = jnp.where(allowed, sc, fill)
                    p = jnp.exp(sc - jnp.max(sc, axis=-1, keepdims=True))
                    l = jnp.sum(p, axis=-1, keepdims=True)
                    os_.append((p.astype(BF16), v, l))
                st[t - D2] = os_
            if 0 <= t - DP < NG:
                os_ = [_dot(p, v)[:SEG + T] / l[:SEG + T] for p, v, l in st[t - DP]]
                o = jnp.concatenate(os_, axis=1)
                ot_v[pl.ds(pl.multiple_of(s * T, T), T), (t - DP) * G * DH:(t - DP + 1) * G * DH] = o[SEG:]
                st[t - DP] = o[:SEG].astype(BF16)
            if 0 <= t - D3 < NG:
                hd = t - D3
                acc = acc + _dot(st.pop(hd), _bf(wo_v[hd * G * DH // 2:(hd + 1) * G * DH // 2, :]))
        m_v[...] = acc[A:]
        ra = pl.ds(r, A)
        b_v[ra, :] = jnp.concatenate([g_v[ra, :]] * (DM // DH), axis=1) * acc[:A] + b_v[ra, :]
        return c

    jax.lax.fori_loop(0, NSEG, step, None)

    ocps = []
    for c in range(EC):
        n = NSEG // EC
        a = _dot(ot_v[c * n * T:(c + 1) * n * T, :].astype(BF16), _bf(wo_v[...]))
        for k in range(n):
            r0 = (c * n + k) * SEG
            gt = jnp.concatenate([g_v[r0 + A:r0 + SEG, :]] * (DM // DH), axis=1)
            tail = gt * a[k * T:(k + 1) * T] + b_v[r0 + A:r0 + SEG, :]
            o_v[r0:r0 + SEG, :] = jnp.concatenate([b_v[r0:r0 + A, :], tail], axis=0).astype(BF16)
        rr = pl.ds(c * n * SEG, n * SEG)
        ocps.append(pltpu.make_async_copy(o_v.at[rr], o_hbm.at[rr], sems.at[7]))
        ocps[-1].start()
    for c in ocps:
        c.wait()


@jax.jit
def pallas_gated_mix__memory_aug_recurrent_mem_tr__glu_gated_geglu__prompt_kernel(
    A_x, A_mem0, A_Wq, A_Wk, A_Wv, A_Wo, A_seg_len, B_x, B_w_gate, B_w_up, B_w_down, gate_w,
):
    anyspec = pl.BlockSpec(memory_space=pl.ANY)
    vspec = pl.BlockSpec(memory_space=pltpu.VMEM)
    out = pl.pallas_call(
        _kernel,
        out_shape=jax.ShapeDtypeStruct((S, DM), A_x.dtype),
        in_specs=[anyspec, vspec] + [anyspec] * 7 + [vspec],
        out_specs=anyspec,
        scratch_shapes=[
            pltpu.VMEM((S, DM), BF16),
            pltpu.VMEM((H // 2, 2, DM // 2, 3 * DH), U32),
            pltpu.VMEM((H // G, DM // 2, 3 * DH * G), U32),
            pltpu.VMEM((H * DH // 2, DM), U32),
            pltpu.VMEM((DF // 2, DM), U32),
            pltpu.VMEM((DF // 2, DM), U32),
            pltpu.VMEM((DF // 2, DM), U32),
            pltpu.VMEM((S, DM), F32),
            pltpu.VMEM((S, DH), F32),
            pltpu.VMEM((NSEG * T, DM), F32),
            pltpu.VMEM((H // G, NSEG, 2 * T, 3 * DH * G), BF16),
            pltpu.VMEM((NSEG * T, H * DH), F32),
            pltpu.VMEM((M, DM), F32),
            pltpu.VMEM((S, DM), BF16),
            pltpu.SemaphoreType.DMA((8,)),
        ],
        compiler_params=pltpu.CompilerParams(vmem_limit_bytes=112 * 2**20),
    )(A_x.reshape(S, DM), A_mem0.reshape(M, DM),
      *[w.reshape(DM // 2, 2, H, DH) for w in (A_Wq, A_Wk, A_Wv)], A_Wo.reshape(H * DH, DM),
      B_w_gate.T, B_w_up.T, B_w_down, gate_w.reshape(1, DM))
    return out.reshape(1, S, DM)
```
